```python
import os as _os
_os.environ.setdefault("JAX_PLATFORMS", "cpu")
import jax
import jax.numpy as jnp

def _softmax(x, axis=-1):
    return jax.nn.softmax(x, axis=axis)
def _gelu(x):
    return jax.nn.gelu(x, approximate=True)
def _silu(x):
    return jax.nn.silu(x)
def _sigmoid(x):
    return jax.nn.sigmoid(x)
def _layernorm(x, axis=-1, eps=1e-5):
    m = jnp.mean(x, axis=axis, keepdims=True)
    v = jnp.var(x, axis=axis, keepdims=True)
    return (x - m) / jnp.sqrt(v + eps)
def _scatter_add(tgt, idx, src, axis=0):
    return tgt.at[idx].add(src)
def _segment_sum(src, seg, n):
    return jax.ops.segment_sum(src, seg, n)
class _Rng:
    def __init__(self, key):
        self._k = key
    def _next(self):
        self._k, sub = jax.random.split(self._k)
        return sub
    def normal(self, shape):
        return jax.random.normal(self._next(), shape, dtype=jnp.bfloat16)
    def randint(self, lo, hi, shape):
        return jax.random.randint(self._next(), shape, lo, hi, dtype=jnp.int32)
    def uniform(self, shape, lo=0.0, hi=1.0):
        return jax.random.uniform(self._next(), shape, jnp.bfloat16, lo, hi)
    def permutation(self, n):
        return jax.random.permutation(self._next(), n)


kernel_name = 'sequential_preLN__sliding_local_dilated__dense_activation_mish__prompt'

def setup_inputs():
    _rng = _Rng(jax.random.key(int.from_bytes(__import__("os").urandom(4), "little")))
    _w = (lambda a: (lambda t: t.astype(jnp.bfloat16) if jnp.issubdtype(t.dtype, jnp.floating) else t)(jnp.asarray(a)))
    def _A_setup():
        B, S, D = 1, 2048, 512
        return {
            "x": _w((lambda *s: _rng.normal(s) * 0.05)(B, S, D)),
            "wqkv": _w((lambda *s: _rng.normal(s) * 0.05)(D, 3 * D)),
            "wo": _w((lambda *s: _rng.normal(s) * 0.05)(D, D)),
        }
    _A_in = _A_setup()

    def _B_setup():
        B, S, D, F = 1, 2048, 512, 1376
        return {
            "x": _w((lambda *s: _rng.normal(s) * 0.05)(B, S, D)),
            "w1": _w((lambda *s: _rng.normal(s) * 1.6)(D, F) * (D ** -0.5)),
            "b1": _w((lambda *s: _rng.normal(s) * 0.1)(F)),
            "w2": _w((lambda *s: _rng.normal(s) * 0.1)(F, D) * (F ** -0.5)),
        }
    _B_in = _B_setup()

    return {
        "A_x": _A_in["x"],
        "A_wqkv": _A_in["wqkv"],
        "A_wo": _A_in["wo"],
        "B_x": _B_in["x"],
        "B_w1": _B_in["w1"],
        "B_b1": _B_in["b1"],
        "B_w2": _B_in["w2"],
    }

def reference(A_x, A_wqkv, A_wo, B_x, B_w1, B_b1, B_w2):
    def _A_ref(x, wqkv, wo):
        B, S, D = x.shape
        H = 32; Dh = D // H
        W, dil = 8, 2
        qkv = (lambda x, *d: x.transpose(*d))((x @ wqkv).reshape(B, S, 3, H, Dh), 2, 0, 3, 1, 4)
        q, k, v = qkv[0], qkv[1], qkv[2]
        scale = Dh ** -0.5
        pos = jnp.arange(S)
        off = jnp.arange(W) * dil
        idx = pos[:, None] - off[None, :]
        mask = idx >= 0
        idx_c = jnp.where(mask, idx, 0).reshape(-1)
        kg = k[:, :, idx_c, :].reshape(B, H, S, W, Dh)
        vg = v[:, :, idx_c, :].reshape(B, H, S, W, Dh)
        logits = jnp.einsum("bhsd,bhswd->bhsw", q, kg) * scale
        logits = jnp.where(mask[None, None, :, :], logits, -1e9)
        attn = _softmax(logits, axis=-1)
        o = jnp.einsum("bhsw,bhswd->bhsd", attn, vg)
        return (lambda x, *d: x.transpose(*d))(o, 0, 2, 1, 3).reshape(B, S, D) @ wo

    def _B_ref(x, w1, b1, w2):
        h = jnp.einsum("bsd,df->bsf", x, w1) + b1
        sp = jnp.log1p(jnp.exp(-jnp.abs(h))) + jnp.where(h > 0, h, jnp.zeros_like(h))
        act = h * jnp.tanh(sp)
        return jnp.einsum("bsf,fd->bsd", act, w2)

    x = A_x
    h = x + _A_ref(_layernorm(x, axis=-1), A_wqkv, A_wo)
    h2 = h + _B_ref(_layernorm(h, axis=-1), B_w1, B_b1, B_w2)
    return h2
```

```python
import functools
import jax
import jax.numpy as jnp
import jax.experimental.pallas as pl
import jax.experimental.pallas.tpu as pltpu

H = 32
DH = 16
W = 8
DIL = 2
HALO = 128
EPS = 1e-5


def _ln(x):
    m = jnp.mean(x, axis=-1, keepdims=True)
    xc = x - m
    v = jnp.mean(xc * xc, axis=-1, keepdims=True)
    return xc * jax.lax.rsqrt(v + EPS)


def _kernel(x_ref, wqkvt_ref, wo_ref, w1_ref, b1_ref, w2_ref, o_ref,
            q_scr, kv_scr, ot_scr, *, T, D):
    i = pl.program_id(0)

    @pl.when(i == 0)
    def _():
        kv_scr[:, 0:HALO] = jnp.zeros((2 * D, HALO), jnp.float32)

    @pl.when(i > 0)
    def _():
        kv_scr[:, 0:HALO] = kv_scr[:, T:T + HALO]

    x = x_ref[...].astype(jnp.float32)
    xn = _ln(x).astype(jnp.bfloat16)
    qkvt = jax.lax.dot_general(wqkvt_ref[...], xn, (((1,), (1,)), ((), ())),
                               preferred_element_type=jnp.float32)
    q_scr[...] = qkvt[0:D] * (DH ** -0.5)
    kv_scr[:, HALO:] = qkvt[D:]

    pos = i * T + jax.lax.broadcasted_iota(jnp.int32, (H, T), 1)

    logits = [jnp.zeros((H, T), jnp.float32) for _ in range(W)]
    for d in range(DH):
        qd = q_scr[d * H:(d + 1) * H, :]
        kd = kv_scr[d * H:(d + 1) * H, :]
        for w in range(W):
            kw = kd if w == 0 else pltpu.roll(kd, DIL * w, 1)
            logits[w] = logits[w] + qd * kw[:, HALO:]
    logits = [jnp.where(pos >= DIL * w, logits[w], -1e9) for w in range(W)]
    mx = functools.reduce(jnp.maximum, logits)
    es = [jnp.exp(l - mx) for l in logits]
    den = functools.reduce(lambda a, b: a + b, es)
    inv = 1.0 / den
    attn = [e * inv for e in es]
    for d in range(DH):
        vd = kv_scr[D + d * H:D + (d + 1) * H, :]
        acc = attn[0] * vd[:, HALO:]
        for w in range(1, W):
            acc = acc + attn[w] * pltpu.roll(vd, DIL * w, 1)[:, HALO:]
        ot_scr[d * H:(d + 1) * H, :] = acc

    o = ot_scr[...].T.astype(jnp.bfloat16)
    h = x + jnp.dot(o, wo_ref[...], preferred_element_type=jnp.float32)
    hn = _ln(h).astype(jnp.bfloat16)
    z = jnp.dot(hn, w1_ref[...], preferred_element_type=jnp.float32)
    z = z + b1_ref[...].astype(jnp.float32)
    sp = jnp.log1p(jnp.exp(-jnp.abs(z))) + jnp.maximum(z, 0.0)
    act = (z * jnp.tanh(sp)).astype(jnp.bfloat16)
    y = h + jnp.dot(act, w2_ref[...], preferred_element_type=jnp.float32)
    o_ref[...] = y.astype(o_ref.dtype)


@jax.jit
def pallas_sequential_preLN__sliding_local_dilated__dense_activation_mish__prompt_kernel(
    A_x: jax.Array,
    A_wqkv: jax.Array,
    A_wo: jax.Array,
    B_x: jax.Array,
    B_w1: jax.Array,
    B_b1: jax.Array,
    B_w2: jax.Array,
):
    B, S, D = A_x.shape
    F = B_w1.shape[1]
    T = 1024
    x2 = A_x.reshape(S, D)
    wqkvt = A_wqkv.reshape(D, 3, H, DH).transpose(1, 3, 2, 0).reshape(3 * D, D)
    wo_p = A_wo.reshape(H, DH, D).transpose(1, 0, 2).reshape(D, D)
    b1 = B_b1.reshape(1, F)
    out = pl.pallas_call(
        functools.partial(_kernel, T=T, D=D),
        grid=(S // T,),
        in_specs=[
            pl.BlockSpec((T, D), lambda i: (i, 0)),
            pl.BlockSpec((3 * D, D), lambda i: (0, 0)),
            pl.BlockSpec((D, D), lambda i: (0, 0)),
            pl.BlockSpec((D, F), lambda i: (0, 0)),
            pl.BlockSpec((1, F), lambda i: (0, 0)),
            pl.BlockSpec((F, D), lambda i: (0, 0)),
        ],
        out_specs=pl.BlockSpec((T, D), lambda i: (i, 0)),
        out_shape=jax.ShapeDtypeStruct((S, D), A_x.dtype),
        scratch_shapes=[
            pltpu.VMEM((D, T), jnp.float32),
            pltpu.VMEM((2 * D, T + HALO), jnp.float32),
            pltpu.VMEM((D, T), jnp.float32),
        ],
        compiler_params=pltpu.CompilerParams(
            dimension_semantics=("arbitrary",),
            vmem_limit_bytes=64 * 1024 * 1024,
        ),
    )(x2, wqkvt, wo_p, B_w1, b1, B_w2)
    return out.reshape(B, S, D)
```
